```python
import os as _os
_os.environ.setdefault("JAX_PLATFORMS", "cpu")
import jax
import jax.numpy as jnp

def _softmax(x, axis=-1):
    return jax.nn.softmax(x, axis=axis)
def _gelu(x):
    return jax.nn.gelu(x, approximate=True)
def _silu(x):
    return jax.nn.silu(x)
def _sigmoid(x):
    return jax.nn.sigmoid(x)
def _layernorm(x, axis=-1, eps=1e-5):
    m = jnp.mean(x, axis=axis, keepdims=True)
    v = jnp.var(x, axis=axis, keepdims=True)
    return (x - m) / jnp.sqrt(v + eps)
def _scatter_add(tgt, idx, src, axis=0):
    return tgt.at[idx].add(src)
def _segment_sum(src, seg, n):
    return jax.ops.segment_sum(src, seg, n)
class _Rng:
    def __init__(self, key):
        self._k = key
    def _next(self):
        self._k, sub = jax.random.split(self._k)
        return sub
    def normal(self, shape):
        return jax.random.normal(self._next(), shape, dtype=jnp.bfloat16)
    def randint(self, lo, hi, shape):
        return jax.random.randint(self._next(), shape, lo, hi, dtype=jnp.int32)
    def uniform(self, shape, lo=0.0, hi=1.0):
        return jax.random.uniform(self._next(), shape, jnp.bfloat16, lo, hi)
    def permutation(self, n):
        return jax.random.permutation(self._next(), n)


kernel_name = 'standalone__cross_network_dcn_v2__recsys'

def setup_inputs():
    _rng = _Rng(jax.random.key(int.from_bytes(__import__("os").urandom(4), "little")))
    _w = (lambda a: (lambda t: t.astype(jnp.bfloat16) if jnp.issubdtype(t.dtype, jnp.floating) else t)(jnp.asarray(a)))
    B, F, D, L = 16384, 26, 16, 6
    Din = min(F * D, 512)
    R = max(Din // 4, 2)
    sc = Din ** -0.5
    return {
        "x0": _w((lambda *s: _rng.normal(s) * 0.05)(B, Din)),
        "U":  _w((lambda *s: _rng.normal(s) * 1.6)(L, Din, R) * sc),
        "V":  _w((lambda *s: _rng.normal(s) * 1.6)(L, R, Din) * sc),
        "bs": _w((lambda *s: _rng.normal(s) * 0.05)(L, Din)),
    }

def reference(x0, U, V, bs):
    x = x0
    for l in range(U.shape[0]):
        h = jnp.einsum('rd,bd->br', V[l], x)
        h = jnp.einsum('dr,br->bd', U[l], h)
        x = x0 * (h + bs[l]) + x
    return x
```

```python
import jax
import jax.numpy as jnp
from jax import lax
import jax.experimental.pallas as pl
import jax.experimental.pallas.tpu as pltpu

_F32 = jnp.float32
_BF16 = jnp.bfloat16


def _dot(a, b):
    return jnp.dot(a, b, preferred_element_type=_F32)


@jax.jit
def pallas_standalone__cross_network_dcn_v2__recsys_kernel(
    x0: jax.Array,
    U: jax.Array,
    V: jax.Array,
    bs: jax.Array,
):
    B, D = x0.shape
    L, _, R = U.shape
    bt, w, skew = 1024, 128, 4
    G = bt // w
    DA = 384

    def kern(x0_ref, u_ref, v_ref, b_ref, o_ref, va_ref, up_ref, vc_ref, x0f_ref, x_ref, z_ref):
        @pl.when(pl.program_id(0) == 0)
        def _():
            bT = b_ref[...].astype(_F32).T
            for l in range(L):
                v = v_ref[l].astype(_F32)
                for k in range(3):
                    va_ref[l, k] = v[:, 128 * k:128 * k + 128]
                vsel = jnp.concatenate([jnp.zeros((R, R + 1), _F32), v[:, DA + 9:]], axis=1)
                p = _dot(u_ref[l], vsel.astype(_BF16))
                u = jnp.concatenate(
                    [u_ref[l].astype(_F32), bT[:, l:l + 1], jnp.zeros((D, 128 - R - 1), _F32)], axis=1)
                lane = lax.broadcasted_iota(jnp.int32, (D, 128), 1)
                up_ref[l] = jnp.where(lane <= R, u, p).astype(up_ref.dtype)
                for j in range(9):
                    vc_ref[l, j] = jnp.broadcast_to(v[:, DA + j:DA + j + 1], (R, 128))

        n = G * L
        for t in range(n + skew):
            if t < n:
                c, l = t % G, t // G
                cs = slice(c * w, (c + 1) * w)
                if l == 0:
                    x0f_ref[c] = x0_ref[:, cs].astype(_F32)
                src = x0f_ref if l == 0 else x_ref
                h = None
                for j in range(9):
                    term = vc_ref[l, j] * src[c, DA + j:DA + j + 1, :]
                    h = term if h is None else h + term
                for k in range(3):
                    if l == 0:
                        rhs = x0_ref[128 * k:128 * k + 128, cs]
                    else:
                        rhs = x_ref[c, 128 * k:128 * k + 128, :].astype(_BF16)
                    h = h + _dot(va_ref[l, k], rhs)
                row = lax.broadcasted_iota(jnp.int32, (8, w), 0)
                z = jnp.concatenate(
                    [h, jnp.where(row == 0, 1.0, src[c, DA + 8:DA + 16, :]), src[c, DA + 16:, :]], axis=0)
                z_ref[c] = z.astype(z_ref.dtype)
            if t >= skew:
                c, l = (t - skew) % G, (t - skew) // G
                cs = slice(c * w, (c + 1) * w)
                src = x0f_ref if l == 0 else x_ref
                bounds = [0, 112, 208, 320, D]
                for r0, r1 in zip(bounds[:-1], bounds[1:]):
                    y = _dot(up_ref[l, r0:r1, :], z_ref[c])
                    xn = x0f_ref[c, r0:r1, :] * y + src[c, r0:r1, :]
                    if l == L - 1:
                        o_ref[r0:r1, cs] = xn.astype(o_ref.dtype)
                    else:
                        x_ref[c, r0:r1, :] = xn

    out = pl.pallas_call(
        kern,
        grid=(B // bt,),
        in_specs=[pl.BlockSpec((D, bt), lambda i: (0, i)),
                  pl.BlockSpec((L, D, R), lambda i: (0, 0, 0)),
                  pl.BlockSpec((L, R, D), lambda i: (0, 0, 0)),
                  pl.BlockSpec((L, D), lambda i: (0, 0))],
        out_specs=pl.BlockSpec((D, bt), lambda i: (0, i)),
        out_shape=jax.ShapeDtypeStruct((D, B), x0.dtype),
        scratch_shapes=[pltpu.VMEM((L, 3, R, 128), _F32),
                        pltpu.VMEM((L, D, 128), _BF16),
                        pltpu.VMEM((L, 9, R, 128), _F32),
                        pltpu.VMEM((G, D, w), _F32),
                        pltpu.VMEM((G, D, w), _F32),
                        pltpu.VMEM((G, 128, w), _BF16)],
        compiler_params=pltpu.CompilerParams(
            dimension_semantics=("arbitrary",), vmem_limit_bytes=100 * 1024 * 1024),
    )(x0.T, U, V, bs)
    return out.T
```

```python
import jax
import jax.numpy as jnp
from jax import lax
import jax.experimental.pallas as pl
import jax.experimental.pallas.tpu as pltpu

_F32 = jnp.float32
_BF16 = jnp.bfloat16
_U32 = jnp.uint32

_W = 128
_PAIR = 2 * _W
_DA = 384
_NC = 9
_N_FIRST = 8
_N_MAIN = 40
_SPLIT = 6
_ROW_CHUNKS = (0, 112, 208, 320, 416)

_FIRST_GROUPS = (
    ("v0",), ("x01",), ("u0", "b"), ("x12",), ("v1",), ("u1",), ("v2", "u2"),
    ("v3", "u3", "v4", "u4", "v5", "u5"), ("x24",),
)
_FIRST_PROGRAM = """
    s0 f s1 f s2 f s3 w0 s4 s5 w1 s6 a0 A10 A00 @A10 w2 pb u0 B00 @B00 w3 s7 A20 A30 @A20 w4 B10
    @B10 w5 s8 a1 A11 A01 B20 B30 u1 A31 A21 B01 B11 @A31 w6 n1 B21 B31 a2 A02 u2 A12 A32 A22 B02
    @B02 w7 n2 a3 B12 B32 B22 u3 A03 A13 a4 A23 A33 B03 B13 B23 A04 B33 A14 u4 @A04 w8 A24 B04 a5
    A40 A34 B14 u5 B24 A50 B34 A05 A15 B40 A70 B50 A60 A25 A41 A35 B60 A51 B05 B15 B41 B25 B70 B35
    A61 A71 B51 A42 B61 B71 A52 A62 A72 B42 B52 B62 A43 B72 A53 A63 A73 B43 B53 B63 A44 B73 A54 A64
    B44 A74 B54 B64 A45 B74 A55 A65 A75 B45 B55 B65 B75
"""


def _parse(text):
    return [("AB".index(t[0]) + 1, int(t[1:-1]), int(t[-1])) if t[0] in "AB" else t
            for t in text.split()]


def _wavefront(n_tiles, n_layers, n_head=6, n_tail=4, skew=4):
    def entry(c):
        lead = n_head // 2 - 1
        return min(max(0, c // 2 - lead), max(0, (n_tiles - n_tail) // 2 - lead))

    tasks = sorted(((c, l) for c in range(n_tiles) for l in range(n_layers)),
                   key=lambda t: (entry(t[0]) + t[1], t[0]))
    pos = {t: i for i, t in enumerate(tasks)}
    due = {}
    for i, (c, l) in enumerate(tasks):
        gap = pos[(c, l + 1)] - i if l + 1 < n_layers else i - pos[(c, l - 1)]
        due.setdefault(i + max(1, min(skew, gap // 2)), []).append((c, l))
    program = []
    for i in range(len(tasks) + skew + 1):
        if i < len(tasks):
            program.append((1,) + tasks[i])
        program.extend((2,) + t for t in due.get(i, []))
    return program


def _dot(a, b):
    return jnp.dot(a, b, preferred_element_type=_F32)


def _pack(a):
    return pltpu.bitcast(a.astype(_BF16), _U32)


def _unpack(a):
    return pltpu.bitcast(a, _BF16)


def _cross_network_kernel(x0_hbm, u_hbm, v_hbm, b_hbm, out_hbm,
                          in_first, in_main, out_buf, u_buf, v_buf, b_buf,
                          va_ref, vc_ref, up_ref, bias_ref, x0_ref, x_ref, z_ref,
                          sem_in, sem_out, sem_first):
    L, D, R = u_hbm.shape
    n_main = (x0_hbm.shape[1] // _W - _N_FIRST) // _N_MAIN
    last_pair = _N_MAIN // 2 - 1

    def cols(pair, n=1):
        start = pair * _PAIR if isinstance(pair, int) else pl.multiple_of(pair * _PAIR, _PAIR)
        return pl.ds(start, n * _PAIR)

    def fetch(slot, pair, sem, n=1):
        return pltpu.make_async_copy(
            x0_hbm.at[:, cols(pair, n)], in_main.at[:, cols(slot, n)], sem_in.at[sem])

    def wait_fetched(slot, sem, n=1):
        filled = in_main.at[:, cols(slot, n)]
        pltpu.make_async_copy(filled, filled, sem_in.at[sem]).wait()

    def first_copy(name, group):
        sem = sem_first.at[group]
        if name == "b":
            return pltpu.make_async_copy(b_hbm, b_buf.at[0], sem)
        if name[0] == "v":
            return pltpu.make_async_copy(v_hbm.at[int(name[1])], v_buf.at[int(name[1])], sem)
        if name[0] == "u":
            return pltpu.make_async_copy(u_hbm.at[int(name[1])], u_buf.at[int(name[1])], sem)
        span = cols(int(name[1]), int(name[2]) - int(name[1]))
        return pltpu.make_async_copy(x0_hbm.at[:, span], in_first.at[:, span], sem)

    def hold_wait(kind, value):
        value = value.astype(_BF16)
        if kind == "v":
            v_buf[L, 0:16, 0:_W] = value
        elif kind == "u":
            u_buf[L, 0:16, :] = value[:, :R]
        elif kind == "b":
            b_buf[1, :, 0:_W] = value[0:L]
        elif kind == "x":
            in_first[0:16, _N_FIRST * _W:(_N_FIRST + 1) * _W] = value
        else:
            in_main[0:16, (_N_MAIN + 2) * _W:(_N_MAIN + 3) * _W] = value

    def prepare_biases():
        rows = jnp.concatenate(
            [jnp.zeros((R, D), _F32), b_buf[0].astype(_F32), jnp.zeros((_W - R - L, D), _F32)], axis=0)
        bias_ref[...] = rows.T

    def prepare_v(l):
        v = v_buf[l].astype(_F32)
        for k in range(_DA // _W):
            va_ref[l, k] = v[:, k * _W:(k + 1) * _W]
        for j in range(_NC):
            vc_ref[l, j] = jnp.broadcast_to(v[:, _DA + j:_DA + j + 1], (R, _W))

    def prepare_u(l):
        v_b = v_buf[l, :, _DA:].astype(_F32)[:, _NC:]
        v_b = jnp.concatenate([jnp.zeros((R, R + 1), _F32), v_b], axis=1)
        v_b = jnp.concatenate([v_b, jnp.zeros((_W - R, _W), _F32)], axis=0)
        k = lax.broadcasted_iota(jnp.int32, (_W, _W), 0)
        n = lax.broadcasted_iota(jnp.int32, (_W, _W), 1)
        rhs = jnp.where(n < R, jnp.where(k == n, 1.0, 0.0),
                        jnp.where(n == R, jnp.where(k == R + l, 1.0, 0.0), v_b)).astype(_BF16)
        lhs = jnp.concatenate([u_buf[l].astype(_F32), bias_ref[:, R:]], axis=1).astype(_BF16)
        for r0, r1 in zip(_ROW_CHUNKS[:-1], _ROW_CHUNKS[1:]):
            up_ref[l, r0 // 2:r1 // 2] = _pack(_dot(lhs[r0:r1], rhs))

    def run_block(program, block=None, zero=None, fence_sem=None):
        first = block is None
        n_tiles = _N_FIRST if first else _N_MAIN
        pair0 = 0 if first else _N_FIRST // 2 + block * (_N_MAIN // 2)
        in_buf = in_first if first else in_main
        parity = None if first else block & 1

        stages = [op for op in program if not isinstance(op, str)]
        order = {op: i for i, op in enumerate(stages)}
        assert len(stages) == len(order) == 2 * n_tiles * L
        assert all(order[(2, c, l)] > order[(1, c, l)]
                   and (l == 0 or order[(1, c, l)] > order[(2, c, l - 1)])
                   for c in range(n_tiles) for l in range(L))
        stage1 = [(c, l) for s, c, l in stages if s == 1]
        arrived = [] if first else list(range(n_tiles))
        converted, results = [], {}

        def refill(p):
            if p == last_pair:
                slot, sem = p + 1 - parity, 3 - parity
            else:
                slot, sem = p + zero * (last_pair + 1 - p), int(p >= _SPLIT)

            @pl.when(block + 1 < n_main)
            def _():
                fetch(slot, pair0 + _N_MAIN // 2 + p, sem).start()

        def convert(p, latest):
            if p in converted:
                return
            converted.append(p)
            if not first and p == _SPLIT:
                hold_wait("main", latest)
                wait_fetched(_SPLIT, 1, last_pair - _SPLIT)
                wait_fetched(last_pair + parity, 2 + parity)
            slot = p + parity if (not first and p == last_pair) else p
            x0 = in_buf[:, cols(slot)].astype(_F32)
            x0_ref[2 * p] = x0[:, :_W]
            x0_ref[2 * p + 1] = x0[:, _W:]
            if not first and p != last_pair:
                refill(p)

        def stage_1(c, l, direct, latest):
            src = x0_ref if l == 0 else x_ref
            parts = []
            for k in range(_DA // _W):
                if direct:
                    rhs = in_buf[k * _W:(k + 1) * _W, c * _W:(c + 1) * _W]
                else:
                    rhs = src[c, k * _W:(k + 1) * _W, :].astype(_BF16)
                parts.append(_dot(va_ref[l, k], rhs))
            if direct:
                convert(c // 2, latest)
            h = vc_ref[l, 0] * src[c, _DA:_DA + 1, :]
            for j in range(1, _NC):
                h = h + vc_ref[l, j] * src[c, _DA + j:_DA + j + 1, :]
            for part in parts:
                h = h + part
            row = lax.broadcasted_iota(jnp.int32, (8, _W), 0)
            one_then_x = jnp.where(row == 0, 1.0, src[c, _DA + 8:_DA + 16, :])
            z_ref[c] = _pack(jnp.concatenate([h, one_then_x, src[c, _DA + 16:, :]], axis=0))
            return h[0:16]

        def stage_2(c, l):
            src = x0_ref if l == 0 else x_ref
            pair, half = pair0 + c // 2, slice((c % 2) * _W, (c % 2 + 1) * _W)
            head = None
            for r0, r1 in zip(_ROW_CHUNKS[:-1], _ROW_CHUNKS[1:]):
                y = _dot(_unpack(up_ref[l, r0 // 2:r1 // 2, :]), _unpack(z_ref[c]))
                x = x0_ref[c, r0:r1, :] * y + src[c, r0:r1, :]
                head = x[0:16] if head is None else head
                if l == L - 1:
                    out_buf[pair, r0:r1, half] = x.astype(out_buf.dtype)
                else:
                    x_ref[c, r0:r1, :] = x
            if l == L - 1 and c % 2 == 1:
                assert order[(2, c - 1, l)] < order[(2, c, l)]
                pltpu.make_async_copy(out_buf.at[pair], out_hbm.at[:, cols(pair)], sem_out).start()
            return head

        if not first:
            wait_fetched(0, 0, _SPLIT)
            refill(last_pair)

        n_stage1, latest, hold = 0, None, None
        for op in program:
            if not isinstance(op, str):
                s, c, l = op
                if s == 2:
                    results[op] = stage_2(c, l)
                    continue
                assert l > 0 or c in arrived
                direct = first and l == 0 and c < 4
                if not direct:
                    for c_next, l_next in stage1[n_stage1:n_stage1 + 6]:
                        if l_next == 0 and c_next in arrived:
                            convert(c_next // 2, latest)
                results[op] = latest = stage_1(c, l, direct, latest)
                n_stage1 += 1
            elif op == "f":
                pl.semaphore_signal(fence_sem, 1)
                pl.semaphore_wait(fence_sem, 1)
            elif op == "n1":
                fetch(0, _N_FIRST // 2, 0, _SPLIT).start()
            elif op == "n2":
                fetch(_SPLIT, _N_FIRST // 2 + _SPLIT, 1, last_pair - _SPLIT).start()
                fetch(last_pair, _N_FIRST // 2 + last_pair, 2).start()
            elif op == "pb":
                prepare_biases()
            elif op[0] == "a":
                prepare_v(int(op[1]))
            elif op[0] == "u":
                prepare_u(int(op[1]))
            elif op[0] == "@":
                hold = results[_parse(op[1:])[0]]
            elif op[0] == "s":
                for name in _FIRST_GROUPS[int(op[1])]:
                    first_copy(name, int(op[1])).start()
            else:
                names = _FIRST_GROUPS[int(op[1])]
                if hold is not None:
                    for name in names:
                        hold_wait(name[0], hold)
                for name in names:
                    first_copy(name, int(op[1])).wait()
                    if name[0] == "x":
                        arrived.extend(range(2 * int(name[1]), 2 * int(name[2])))
                hold = None

    def block_body(s, carry):
        @pl.when(s == 0)
        def _():
            pl.run_scoped(lambda sem: run_block(_parse(_FIRST_PROGRAM), fence_sem=sem),
                          pltpu.SemaphoreType.REGULAR)

        @pl.when(s > 0)
        def _():
            run_block(_wavefront(_N_MAIN, L), block=s - 1, zero=(s * (s - 1)) & 1)

        return carry

    lax.fori_loop(0, n_main + 1, block_body, 0)
    pltpu.make_async_copy(out_buf, out_buf, sem_out).wait()


@jax.jit
def pallas_standalone__cross_network_dcn_v2__recsys_kernel(
    x0: jax.Array,
    U: jax.Array,
    V: jax.Array,
    bs: jax.Array,
):
    B, D = x0.shape
    L, _, R = U.shape
    assert (L, D, R) == (6, _ROW_CHUNKS[-1], _W - (D - _DA - _NC) - 1)
    assert B % _W == 0 and (B // _W - _N_FIRST) > 0 and (B // _W - _N_FIRST) % _N_MAIN == 0
    hbm = pl.BlockSpec(memory_space=pl.ANY)
    out = pl.pallas_call(
        _cross_network_kernel,
        in_specs=[hbm, hbm, hbm, hbm],
        out_specs=hbm,
        out_shape=jax.ShapeDtypeStruct((D, B), x0.dtype),
        scratch_shapes=[
            pltpu.VMEM((D, (_N_FIRST + 2) * _W), x0.dtype),
            pltpu.VMEM((D, (_N_MAIN + 6) * _W), x0.dtype),
            pltpu.VMEM((B // _PAIR, D, _PAIR), x0.dtype),
            pltpu.VMEM((L + 1, D, R), U.dtype),
            pltpu.VMEM((L + 1, R, D), V.dtype),
            pltpu.VMEM((2, L, D), bs.dtype),
            pltpu.VMEM((L, _DA // _W, R, _W), _F32),
            pltpu.VMEM((L, _NC, R, _W), _F32),
            pltpu.VMEM((L, D // 2, _W), _U32),
            pltpu.VMEM((D, _W), _F32),
            pltpu.VMEM((_N_MAIN, D, _W), _F32),
            pltpu.VMEM((_N_MAIN, D, _W), _F32),
            pltpu.VMEM((_N_MAIN, _W // 2, _W), _U32),
            pltpu.SemaphoreType.DMA((4,)),
            pltpu.SemaphoreType.DMA,
            pltpu.SemaphoreType.DMA((len(_FIRST_GROUPS),)),
        ],
        compiler_params=pltpu.CompilerParams(
            vmem_limit_bytes=80 * 1024 * 1024,
            disable_bounds_checks=True,
            disable_semaphore_checks=True,
            flags={"XLA_TPU_RESCHEDULE_DMA_DONES": True},
        ),
    )(x0.T, U, V, bs)
    return out.T
```

```python
import jax
import jax.numpy as jnp
from jax import lax
import jax.experimental.pallas as pl
import jax.experimental.pallas.tpu as pltpu

_F32 = jnp.float32
_BF16 = jnp.bfloat16
_U32 = jnp.uint32

_W = 128
_PAIR = 2 * _W
_DA = 384
_NC = 9
_N_FIRST = 8
_N_MAIN = 40
_SPLIT = 6
_ROW_CHUNKS = (0, 112, 208, 320, 416)

_FIRST_GROUPS = (
    ("v0",), ("x01",), ("u0", "b"), ("x12",), ("v1",), ("u1",), ("v2", "u2"),
    ("v3", "u3", "v4", "u4", "v5", "u5"), ("x24",),
)
_FIRST_PROGRAM = """
    s0 s1 s2 s3 w0 s4 s5 w1 s6 a0 A10 A00 @A10 w2 pb u0 B00 @B00 w3 s7 A20 A30 @A20 w4 B10
    @B10 w5 s8 a1 A11 A01 B20 B30 u1 A31 A21 B01 B11 @A31 w6 n1 B21 B31 a2 A02 u2 A12 A32 A22 B02
    @B02 w7 n2 a3 B12 B32 B22 u3 A03 A13 a4 A23 A33 B03 B13 B23 A04 B33 A14 u4 @A04 w8 A24 B04 a5
    A40 A34 B14 u5 B24 A50 B34 A05 A15 B40 A70 B50 A60 A25 A41 A35 B60 A51 B05 B15 B41 B25 B70 B35
    A61 A71 B51 A42 B61 B71 A52 A62 A72 B42 B52 B62 A43 B72 A53 A63 A73 B43 B53 B63 A44 B73 A54 A64
    B44 A74 B54 B64 A45 B74 A55 A65 A75 B45 B55 B65 B75
"""


def _parse(text):
    return [("AB".index(t[0]) + 1, int(t[1:-1]), int(t[-1])) if t[0] in "AB" else t
            for t in text.split()]


def _wavefront(n_tiles, n_layers, n_head=6, n_tail=4, skew=4):
    def entry(c):
        lead = n_head // 2 - 1
        return min(max(0, c // 2 - lead), max(0, (n_tiles - n_tail) // 2 - lead))

    tasks = sorted(((c, l) for c in range(n_tiles) for l in range(n_layers)),
                   key=lambda t: (entry(t[0]) + t[1], t[0]))
    pos = {t: i for i, t in enumerate(tasks)}
    due = {}
    for i, (c, l) in enumerate(tasks):
        gap = pos[(c, l + 1)] - i if l + 1 < n_layers else i - pos[(c, l - 1)]
        due.setdefault(i + max(1, min(skew, gap // 2)), []).append((c, l))
    program = []
    for i in range(len(tasks) + skew + 1):
        if i < len(tasks):
            program.append((1,) + tasks[i])
        program.extend((2,) + t for t in due.get(i, []))
    return program


def _dot(a, b):
    return jnp.dot(a, b, preferred_element_type=_F32)


def _pack(a):
    return pltpu.bitcast(a.astype(_BF16), _U32)


def _unpack(a):
    return pltpu.bitcast(a, _BF16)


def _cross_network_kernel(x0_hbm, u_hbm, v_hbm, b_hbm, out_hbm,
                          in_first, in_main, out_buf, u_buf, v_buf, b_buf,
                          va_ref, vc_ref, up_ref, bias_ref, x0_ref, x_ref, z_ref,
                          sem_in, sem_out, sem_first):
    L, D, R = u_hbm.shape
    n_main = (x0_hbm.shape[1] // _W - _N_FIRST) // _N_MAIN
    last_pair = _N_MAIN // 2 - 1

    def cols(pair, n=1):
        start = pair * _PAIR if isinstance(pair, int) else pl.multiple_of(pair * _PAIR, _PAIR)
        return pl.ds(start, n * _PAIR)

    def fetch(slot, pair, sem, n=1):
        return pltpu.make_async_copy(
            x0_hbm.at[:, cols(pair, n)], in_main.at[:, cols(slot, n)], sem_in.at[sem])

    def wait_fetched(slot, sem, n=1):
        filled = in_main.at[:, cols(slot, n)]
        pltpu.make_async_copy(filled, filled, sem_in.at[sem]).wait()

    def first_copy(name, group):
        sem = sem_first.at[group]
        if name == "b":
            return pltpu.make_async_copy(b_hbm, b_buf, sem)
        if name[0] == "v":
            return pltpu.make_async_copy(v_hbm.at[int(name[1])], v_buf.at[int(name[1])], sem)
        if name[0] == "u":
            return pltpu.make_async_copy(u_hbm.at[int(name[1])], u_buf.at[int(name[1])], sem)
        span = cols(int(name[1]), int(name[2]) - int(name[1]))
        return pltpu.make_async_copy(x0_hbm.at[:, span], in_first.at[:, span], sem)

    def hold_wait(kind, value):
        value = value.astype(_BF16)
        if kind == "v":
            v_buf[L, 0:16, 0:_W] = value
        elif kind == "u":
            u_buf[L, 0:16, :] = value[:, :R]
        elif kind == "x":
            in_first[0:16, _N_FIRST * _W:(_N_FIRST + 1) * _W] = value
        else:
            in_main[0:16, (_N_MAIN + 2) * _W:(_N_MAIN + 3) * _W] = value

    def prepare_biases():
        rows = jnp.concatenate(
            [jnp.zeros((R, D), _F32), b_buf[...].astype(_F32), jnp.zeros((_W - R - L, D), _F32)], axis=0)
        bias_ref[...] = rows.T

    def prepare_v(l):
        v = v_buf[l].astype(_F32)
        for k in range(_DA // _W):
            va_ref[l, k] = v[:, k * _W:(k + 1) * _W]
        for j in range(_NC):
            vc_ref[l, j, 0:R] = jnp.broadcast_to(v[:, _DA + j:_DA + j + 1], (R, _W))

    def prepare_u(l):
        v_b = v_buf[l, :, _DA:].astype(_F32)[:, _NC:]
        v_b = jnp.concatenate([jnp.zeros((R, R + 1), _F32), v_b], axis=1)
        v_b = jnp.concatenate([v_b, jnp.zeros((_W - R, _W), _F32)], axis=0)
        k = lax.broadcasted_iota(jnp.int32, (_W, _W), 0)
        n = lax.broadcasted_iota(jnp.int32, (_W, _W), 1)
        rhs = jnp.where(n < R, jnp.where(k == n, 1.0, 0.0),
                        jnp.where(n == R, jnp.where(k == R + l, 1.0, 0.0), v_b)).astype(_BF16)
        lhs = jnp.concatenate([u_buf[l].astype(_F32), bias_ref[:, R:]], axis=1).astype(_BF16)
        for r0, r1 in zip(_ROW_CHUNKS[:-1], _ROW_CHUNKS[1:]):
            up_ref[l, r0 // 2:r1 // 2] = _pack(_dot(lhs[r0:r1], rhs))

    def run_block(program, block=None, zero=None):
        first = block is None
        n_tiles = _N_FIRST if first else _N_MAIN
        pair0 = 0 if first else _N_FIRST // 2 + block * (_N_MAIN // 2)
        in_buf = in_first if first else in_main
        parity = None if first else block & 1

        stages = [op for op in program if not isinstance(op, str)]
        order = {op: i for i, op in enumerate(stages)}
        assert len(stages) == len(order) == 2 * n_tiles * L
        assert all(order[(2, c, l)] > order[(1, c, l)]
                   and (l == 0 or order[(1, c, l)] > order[(2, c, l - 1)])
                   for c in range(n_tiles) for l in range(L))
        stage1 = [(c, l) for s, c, l in stages if s == 1]
        arrived = [] if first else list(range(n_tiles))
        converted, results = [], {}

        def refill(p):
            if p == last_pair:
                slot, sem = p + 1 - parity, 3 - parity
            else:
                slot, sem = p + zero * (last_pair + 1 - p), int(p >= _SPLIT)

            @pl.when(block + 1 < n_main)
            def _():
                fetch(slot, pair0 + _N_MAIN // 2 + p, sem).start()

        def convert(p, latest):
            if p in converted:
                return
            converted.append(p)
            if not first and p == _SPLIT:
                hold_wait("main", latest)
                wait_fetched(_SPLIT, 1, last_pair - _SPLIT)
                wait_fetched(last_pair + parity, 2 + parity)
            slot = p + parity if (not first and p == last_pair) else p
            x0 = in_buf[:, cols(slot)].astype(_F32)
            x0_ref[2 * p, 0:D] = x0[:, :_W]
            x0_ref[2 * p + 1, 0:D] = x0[:, _W:]
            if not first and p != last_pair:
                refill(p)

        def stage_1(c, l, direct, latest):
            src = x0_ref if l == 0 else x_ref
            parts = []
            for k in range(_DA // _W):
                if direct:
                    rhs = in_buf[k * _W:(k + 1) * _W, c * _W:(c + 1) * _W]
                else:
                    rhs = src[c, k * _W:(k + 1) * _W, :].astype(_BF16)
                parts.append(_dot(va_ref[l, k], rhs))
            if direct:
                convert(c // 2, latest)
            h = vc_ref[l, 0, 0:R] * src[c, _DA:_DA + 1, :]
            for j in range(1, _NC):
                h = h + vc_ref[l, j, 0:R] * src[c, _DA + j:_DA + j + 1, :]
            for part in parts:
                h = h + part
            row = lax.broadcasted_iota(jnp.int32, (8, _W), 0)
            one_then_x = jnp.where(row == 0, 1.0, src[c, _DA + 8:_DA + 16, :])
            z = jnp.concatenate([h, one_then_x, src[c, _DA + 16:D, :]], axis=0)
            z_ref[c, 0:_W // 2] = _pack(z)
            return h[0:16]

        def stage_2(c, l):
            src = x0_ref if l == 0 else x_ref
            pair, half = pair0 + c // 2, slice((c % 2) * _W, (c % 2 + 1) * _W)
            head = None
            for r0, r1 in zip(_ROW_CHUNKS[:-1], _ROW_CHUNKS[1:]):
                y = _dot(_unpack(up_ref[l, r0 // 2:r1 // 2, :]), _unpack(z_ref[c, 0:_W // 2]))
                x = x0_ref[c, r0:r1, :] * y + src[c, r0:r1, :]
                head = x[0:16] if head is None else head
                if l == L - 1:
                    out_buf[pair, r0:r1, half] = x.astype(out_buf.dtype)
                else:
                    x_ref[c, r0:r1, :] = x
            if l == L - 1 and c % 2 == 1:
                assert order[(2, c - 1, l)] < order[(2, c, l)]
                pltpu.make_async_copy(out_buf.at[pair], out_hbm.at[:, cols(pair)], sem_out).start()
            return head

        if not first:
            wait_fetched(0, 0, _SPLIT)
            refill(last_pair)

        n_stage1, latest, hold = 0, None, None
        for op in program:
            if not isinstance(op, str):
                s, c, l = op
                if s == 2:
                    results[op] = stage_2(c, l)
                    continue
                assert l > 0 or c in arrived
                direct = first and l == 0 and c < 4
                if not direct:
                    for c_next, l_next in stage1[n_stage1:n_stage1 + 3]:
                        if l_next == 0 and c_next in arrived:
                            convert(c_next // 2, latest)
                results[op] = latest = stage_1(c, l, direct, latest)
                n_stage1 += 1
            elif op == "n1":
                fetch(0, _N_FIRST // 2, 0, _SPLIT).start()
            elif op == "n2":
                fetch(_SPLIT, _N_FIRST // 2 + _SPLIT, 1, last_pair - _SPLIT).start()
                fetch(last_pair, _N_FIRST // 2 + last_pair, 2).start()
            elif op == "pb":
                prepare_biases()
            elif op[0] == "a":
                prepare_v(int(op[1]))
            elif op[0] == "u":
                prepare_u(int(op[1]))
            elif op[0] == "@":
                hold = results[_parse(op[1:])[0]]
            elif op[0] == "s":
                for name in _FIRST_GROUPS[int(op[1])]:
                    first_copy(name, int(op[1])).start()
            else:
                names = _FIRST_GROUPS[int(op[1])]
                if hold is not None:
                    hold_wait(names[0][0], hold)
                for name in names:
                    first_copy(name, int(op[1])).wait()
                    if name[0] == "x":
                        arrived.extend(range(2 * int(name[1]), 2 * int(name[2])))
                hold = None

    def block_body(s, carry):
        @pl.when(s == 0)
        def _():
            run_block(_parse(_FIRST_PROGRAM))

        @pl.when(s > 0)
        def _():
            run_block(_wavefront(_N_MAIN, L), block=s - 1, zero=(s * (s - 1)) & 1)

        return carry

    lax.fori_loop(0, n_main + 1, block_body, 0)
    pltpu.make_async_copy(out_buf, out_buf, sem_out).wait()


@jax.jit
def pallas_standalone__cross_network_dcn_v2__recsys_kernel(
    x0: jax.Array,
    U: jax.Array,
    V: jax.Array,
    bs: jax.Array,
):
    B, D = x0.shape
    L, _, R = U.shape
    assert (L, D, R) == (6, _ROW_CHUNKS[-1], _W - (D - _DA - _NC) - 1)
    assert B % _W == 0 and (B // _W - _N_FIRST) > 0 and (B // _W - _N_FIRST) % _N_MAIN == 0
    hbm = pl.BlockSpec(memory_space=pl.ANY)
    out = pl.pallas_call(
        _cross_network_kernel,
        in_specs=[hbm, hbm, hbm, hbm],
        out_specs=hbm,
        out_shape=jax.ShapeDtypeStruct((D, B), x0.dtype),
        scratch_shapes=[
            pltpu.VMEM((D, (_N_FIRST + 2) * _W), x0.dtype),
            pltpu.VMEM((D, (_N_MAIN + 6) * _W), x0.dtype),
            pltpu.VMEM((B // _PAIR, D, _PAIR), x0.dtype),
            pltpu.VMEM((L + 1, D, R), U.dtype),
            pltpu.VMEM((L + 1, R, D), V.dtype),
            pltpu.VMEM((L, D), bs.dtype),
            pltpu.VMEM((L, _DA // _W, R, _W), _F32),
            pltpu.VMEM((L, _NC, R + 24, _W), _F32),
            pltpu.VMEM((L, D // 2 + 8, _W), _U32),
            pltpu.VMEM((D, _W), _F32),
            pltpu.VMEM((_N_MAIN, D + 24, _W), _F32),
            pltpu.VMEM((_N_MAIN, D + 8, _W), _F32),
            pltpu.VMEM((_N_MAIN, _W // 2 + 24, _W), _U32),
            pltpu.SemaphoreType.DMA((4,)),
            pltpu.SemaphoreType.DMA,
            pltpu.SemaphoreType.DMA((len(_FIRST_GROUPS),)),
        ],
        compiler_params=pltpu.CompilerParams(
            vmem_limit_bytes=80 * 1024 * 1024,
            disable_bounds_checks=True,
            disable_semaphore_checks=True,
            flags={"XLA_TPU_RESCHEDULE_DMA_DONES": True},
        ),
    )(x0.T, U, V, bs)
    return out.T
```
